```python
import jax
import jax.numpy as jnp

def _softmax(x, axis=-1):
    return jax.nn.softmax(x, axis=axis)
def _gelu(x):
    return jax.nn.gelu(x, approximate=True)
def _silu(x):
    return jax.nn.silu(x)
def _sigmoid(x):
    return jax.nn.sigmoid(x)
def _layernorm(x, axis=-1, eps=1e-5):
    m = jnp.mean(x, axis=axis, keepdims=True)
    v = jnp.var(x, axis=axis, keepdims=True)
    return (x - m) / jnp.sqrt(v + eps)
def _scatter_add(tgt, idx, src, axis=0):
    return tgt.at[idx].add(src)
def _segment_sum(src, seg, n):
    return jax.ops.segment_sum(src, seg, n)
class _Rng:
    def __init__(self, key):
        self._k = key
    def _next(self):
        self._k, sub = jax.random.split(self._k)
        return sub
    def normal(self, shape):
        return jax.random.normal(self._next(), shape, dtype=jnp.bfloat16)
    def randint(self, lo, hi, shape):
        return jax.random.randint(self._next(), shape, lo, hi, dtype=jnp.int32)
    def uniform(self, shape, lo=0.0, hi=1.0):
        return jax.random.uniform(self._next(), shape, jnp.bfloat16, lo, hi)
    def permutation(self, n):
        return jax.random.permutation(self._next(), n)


kernel_name = 'gated_mix__sliding_block_cached__glu_gated_swiglu__decode'

def setup_inputs():
    _rng = _Rng(jax.random.key(int.from_bytes(__import__("os").urandom(4), "little")))
    _w = (lambda a: (lambda t: t.astype(jnp.bfloat16) if jnp.issubdtype(t.dtype, jnp.floating) else t)(jnp.asarray(a)))
    def _A_setup():
        B, Sq, D = 1, 1, 640
        Hq, Hkv, Sk, Dh = 32, 32, 32768, 192
        assert Hq % Hkv == 0, (Hq, Hkv)
        return {
            "x": _w((lambda *s: _rng.normal(s) * 0.05)(B, Sq, D)),
            "k_cache": _w((lambda *s: _rng.normal(s) * 0.05)(B, Hkv, Sk, Dh)),
            "v_cache": _w((lambda *s: _rng.normal(s) * 0.05)(B, Hkv, Sk, Dh)),
            "wq": _w((lambda *s: _rng.normal(s) * 0.05)(D, Hq * Dh) * (D ** -0.5)),
            "wo": _w((lambda *s: _rng.normal(s) * 0.05)(Hq * Dh, D) * ((Hq * Dh) ** -0.5)),
        }
    _A_in = _A_setup()

    def _B_setup():
        B, S, D, F = 1, 1, 640, 1536
        return {
            "x": _w((lambda *s: _rng.normal(s) * 0.05)(B, S, D)),
            "w1": _w((lambda *s: _rng.normal(s) * 0.05)(D, F) * (2.0 / D) ** 0.5),
            "w3": _w((lambda *s: _rng.normal(s) * 0.05)(D, F) * (2.0 / D) ** 0.5),
            "w2": _w((lambda *s: _rng.normal(s) * 0.05)(F, D) * (2.0 / F) ** 0.5),
        }
    _B_in = _B_setup()

    return {
        "A_x": _A_in["x"],
        "A_k_cache": _A_in["k_cache"],
        "A_v_cache": _A_in["v_cache"],
        "A_wq": _A_in["wq"],
        "A_wo": _A_in["wo"],
        "B_x": _B_in["x"],
        "B_w1": _B_in["w1"],
        "B_w3": _B_in["w3"],
        "B_w2": _B_in["w2"],
        "gate_w": _w((lambda *s: _rng.normal(s) * 0.05)(640)),
    }

def reference(A_x, A_k_cache, A_v_cache, A_wq, A_wo, B_x, B_w1, B_w3, B_w2, gate_w):
    def _A_ref(x, k_cache, v_cache, wq, wo):
        B, Sq, D = x.shape
        Hq, Dh = 32, 192
        Hkv, Sk = k_cache.shape[1], k_cache.shape[2]
        W = min(4096, max(256, Sk // 4))
        rep = Hq // Hkv
        q = (lambda x, *d: x.transpose(*d))((x @ wq).reshape(B, Sq, Hq, Dh), 0, 2, 1, 3)
        k = jnp.repeat(k_cache[:, :, Sk - W:, :], rep, axis=1)
        v = jnp.repeat(v_cache[:, :, Sk - W:, :], rep, axis=1)
        scores = jnp.einsum("bhqd,bhkd->bhqk", q, k) * (Dh ** -0.5)
        p = _softmax(scores, axis=-1)
        o = jnp.einsum("bhqk,bhkd->bhqd", p, v)
        return (lambda x, *d: x.transpose(*d))(o, 0, 2, 1, 3).reshape(B, Sq, Hq * Dh) @ wo

    def _B_ref(x, w1, w3, w2):
        gate = jnp.einsum("bsd,df->bsf", x, w1)
        up = jnp.einsum("bsd,df->bsf", x, w3)
        h = _silu(gate) * up
        out = jnp.einsum("bsf,fd->bsd", h, w2)
        return out

    x = A_x
    g = _sigmoid((x * gate_w).sum(-1, keepdims=True))
    a = _A_ref(x, A_k_cache, A_v_cache, A_wq, A_wo)
    b = _B_ref(x, B_w1, B_w3, B_w2)
    return g * a + (1 - g) * b
```

```python
import functools
import jax, jax.numpy as jnp
import jax.experimental.pallas as pl
import jax.experimental.pallas.tpu as pltpu

H, DH, W, D, F = 32, 192, 4096, 640, 1536

def kern(x_ref, gw_ref, k_ref, v_ref, wq_ref, wo_ref, w1_ref, w3_ref, w2_ref, o_ref, q_s, acc_s):
    h = pl.program_id(0)
    x = x_ref[0]
    @pl.when(h == 0)
    def _():
        acc_s[...] = jnp.zeros_like(acc_s)
    x8 = jnp.broadcast_to(x, (8, D))
    q2 = jnp.dot(x8, wq_ref[...], preferred_element_type=jnp.float32)
    outs = []
    for j in range(2):
        q = q2[:, j * DH:(j + 1) * DH].astype(jnp.bfloat16)
        s = jnp.dot(q, k_ref[0, j], preferred_element_type=jnp.float32) * (DH ** -0.5)
        m = jnp.max(s, axis=-1, keepdims=True)
        p = jnp.exp(s - m)
        l = jnp.sum(p, axis=-1, keepdims=True)
        o = jax.lax.dot_general(p.astype(jnp.bfloat16), v_ref[0, j], (((1,), (1,)), ((), ())),
                                preferred_element_type=jnp.float32)
        outs.append(o / l)
    o2 = jnp.concatenate(outs, axis=1).astype(jnp.bfloat16)
    acc_s[...] += jnp.dot(o2, wo_ref[...], preferred_element_type=jnp.float32)
    @pl.when(h == pl.num_programs(0) - 1)
    def _():
        gate = jnp.dot(x8, w1_ref[...], preferred_element_type=jnp.float32)
        up = jnp.dot(x8, w3_ref[...], preferred_element_type=jnp.float32)
        hh = (gate * jax.nn.sigmoid(gate) * up).astype(jnp.bfloat16)
        b = jnp.dot(hh, w2_ref[...], preferred_element_type=jnp.float32)
        gw = gw_ref[...].astype(jnp.float32).reshape(1, D)
        g = jax.nn.sigmoid(jnp.sum(x.astype(jnp.float32) * gw, axis=-1, keepdims=True))
        res = g * acc_s[...] + (1 - g) * b
        o_ref[0] = res[0:1].astype(o_ref.dtype)

@jax.jit
def pallas_gated_mix__sliding_block_cached__glu_gated_swiglu__decode_kernel(A_x, A_k_cache, A_v_cache, A_wq, A_wo, B_x, B_w1, B_w3, B_w2, gate_w):
    kT = jnp.swapaxes(A_k_cache, 2, 3)
    vT = jnp.swapaxes(A_v_cache, 2, 3)
    Sk = kT.shape[3]
    last = Sk // W - 1
    full = lambda s: pl.BlockSpec(s, lambda h: (0,) * len(s))
    return pl.pallas_call(
        kern,
        grid=(H // 2,),
        in_specs=[full((1, 1, D)), full((D,)),
                  pl.BlockSpec((1, 2, DH, W), lambda h: (0, h, 0, last)),
                  pl.BlockSpec((1, 2, DH, W), lambda h: (0, h, 0, last)),
                  pl.BlockSpec((D, 2 * DH), lambda h: (0, h)),
                  pl.BlockSpec((2 * DH, D), lambda h: (h, 0)),
                  full((D, F)), full((D, F)), full((F, D))],
        out_specs=full((1, 1, D)),
        out_shape=jax.ShapeDtypeStruct((1, 1, D), jnp.bfloat16),
        scratch_shapes=[pltpu.VMEM((8, H * DH), jnp.float32), pltpu.VMEM((8, D), jnp.float32)],
        compiler_params=pltpu.CompilerParams(dimension_semantics=("arbitrary",), vmem_limit_bytes=100 * 1024 * 1024),
    )(A_x, gate_w, kT, vT, A_wq, A_wo, B_w1, B_w3, B_w2)
```

```python
import jax, jax.numpy as jnp
import jax.experimental.pallas as pl
import jax.experimental.pallas.tpu as pltpu

H, DH, W, D, F = 32, 192, 4096, 640, 1536
BF = jnp.bfloat16
F32 = jnp.float32


def pieces(shape, pr, pc, r0=0, nr=None):
    R, C = shape
    nr = R - r0 if nr is None else nr
    assert nr % pr == 0 and C % pc == 0, (shape, pr, pc, nr)
    return [(r, c) for r in range(r0, r0 + nr, pr) for c in range(0, C, pc)]


def make(NB=2, kv=(192, 128), wq_p=(8, 3072), wo_p=(32, 640), w13_p=(16, 1536), w2_p=(32, 640),
         w2_groups=(512, 512, 384, 128), semcheck=False, bchk=False):
    assert sum(w2_groups) == F
    w2_offs = [sum(w2_groups[:i]) for i in range(len(w2_groups))]
    NG = len(w2_groups)
    S_K, S_V = 0, NB
    S_X = 2 * NB
    S_GW, S_WQ, S_WO, S_W1, S_W3, S_W2 = S_X + 1, S_X + 2, S_X + 3, S_X + 4, S_X + 5, S_X + 6
    NSEM = S_W2 + NG

    def kern(x_hbm, gw_hbm, k_hbm, v_hbm, wq_hbm, wo_hbm, w1_hbm, w3_hbm, w2_hbm, o_ref,
             x_s, gw_s, kbuf, vbuf, wq_s, wo_s, w1_s, w3_s, w2_s, q_s, acc_s, sem):
        SK = k_hbm.shape[3]

        def wpieces(src, dst, p, s, r0=0, nr=None):
            return [pltpu.make_async_copy(src.at[pl.ds(r, p[0]), pl.ds(c, p[1])],
                                          dst.at[pl.ds(r, p[0]), pl.ds(c, p[1])], sem.at[s])
                    for r, c in pieces(dst.shape, p[0], p[1], r0, nr)]

        def start_alt(a, b):
            n = max(len(a), len(b))
            ia = ib = 0
            for i in range(n):
                while ia < len(a) and ia * n < (i + 1) * len(a):
                    a[ia].start(priority=0); ia += 1
                while ib < len(b) and ib * n < (i + 1) * len(b):
                    b[ib].start(priority=1); ib += 1

        def wait_all(buf, s):
            pltpu.make_async_copy(buf, buf, sem.at[s]).wait()

        def kv_pieces(src, buf, h, slot, s):
            out = []
            for c in range(0, W, kv[1]):
                for r in range(0, DH, kv[0]):
                    out.append(pltpu.make_async_copy(
                        src.at[0, h, pl.ds(r, kv[0]), pl.ds(SK - W + c, kv[1])],
                        buf.at[slot, pl.ds(r, kv[0]), pl.ds(c, kv[1])], sem.at[s + slot]))
            return out

        def start_head(h, slot):
            start_alt(kv_pieces(k_hbm, kbuf, h, slot, S_K), kv_pieces(v_hbm, vbuf, h, slot, S_V))

        def start_ffn():
            start_alt(wpieces(w1_hbm, w1_s, w13_p, S_W1), wpieces(w3_hbm, w3_s, w13_p, S_W3))
            for i, (o, n) in enumerate(zip(w2_offs, w2_groups)):
                ps = wpieces(w2_hbm, w2_s, w2_p, S_W2 + i, o, n)
                start_alt(ps[0::2], ps[1::2])

        x_cp = pltpu.make_async_copy(x_hbm, x_s, sem.at[S_X])
        gw_cp = pltpu.make_async_copy(gw_hbm, gw_s, sem.at[S_GW])
        x_cp.start()
        gw_cp.start(priority=1)
        start_alt(wpieces(wq_hbm, wq_s, wq_p, S_WQ), wpieces(wo_hbm, wo_s, wo_p, S_WO))
        start_head(0, 0)

        x_cp.wait()
        x = x_s[0]
        x8 = jnp.broadcast_to(x, (8, D))
        wait_all(wq_s, S_WQ)
        for hp in range(H // 2):
            q2 = jnp.dot(x8, wq_s[:, hp * 2 * DH:(hp + 1) * 2 * DH], preferred_element_type=F32)
            q_s[2 * hp] = q2[:, :DH].astype(BF)
            q_s[2 * hp + 1] = q2[:, DH:].astype(BF)
        acc_s[...] = jnp.zeros_like(acc_s)
        for h in range(1, NB):
            start_head(h, h)
        wait_all(wo_s, S_WO)

        def head(h, carry):
            slot = jax.lax.rem(h, NB)
            wait_all(kbuf.at[slot], S_K + slot)
            s = jnp.dot(q_s[h], kbuf[slot], preferred_element_type=F32) * (DH ** -0.5)
            m = jnp.max(s, axis=-1, keepdims=True)
            p = jnp.exp(s - m)
            l = jnp.sum(p, axis=-1, keepdims=True)
            pb = p.astype(BF)
            wait_all(vbuf.at[slot], S_V + slot)
            o = jax.lax.dot_general(pb, vbuf[slot], (((1,), (1,)), ((), ())), preferred_element_type=F32)
            ob = (o / l).astype(BF)
            row = pl.multiple_of(h * DH, DH)
            acc_s[...] += jnp.dot(ob, wo_s[pl.ds(row, DH), :], preferred_element_type=F32)

            @pl.when(h + NB < H)
            def _():
                start_head(h + NB, slot)

            @pl.when(h + NB == H)
            def _():
                start_ffn()
            return carry

        jax.lax.fori_loop(0, H, head, 0)

        gw_cp.wait()
        gw = gw_s[...].astype(F32).reshape(1, D)
        g = jax.nn.sigmoid(jnp.sum(x.astype(F32) * gw, axis=-1, keepdims=True))
        ga = g * acc_s[...]
        wait_all(w1_s, S_W1)
        gate = jnp.dot(x8, w1_s[...], preferred_element_type=F32)
        sg = gate * jax.nn.sigmoid(gate)
        wait_all(w3_s, S_W3)
        up = jnp.dot(x8, w3_s[...], preferred_element_type=F32)
        hh = (sg * up).astype(BF)
        b = None
        for i, (o, n) in enumerate(zip(w2_offs, w2_groups)):
            wait_all(w2_s.at[pl.ds(o, n)], S_W2 + i)
            part = jnp.dot(hh[:, o:o + n], w2_s[o:o + n, :], preferred_element_type=F32)
            b = part if b is None else b + part
        res = ga + (1 - g) * b
        o_ref[0] = res[0:1].astype(o_ref.dtype)

    @jax.jit
    def f(A_x, A_k_cache, A_v_cache, A_wq, A_wo, B_x, B_w1, B_w3, B_w2, gate_w):
        kT = jnp.swapaxes(A_k_cache, 2, 3)
        vT = jnp.swapaxes(A_v_cache, 2, 3)
        anyspec = pl.BlockSpec(memory_space=pl.ANY)
        return pl.pallas_call(
            kern,
            in_specs=[anyspec] * 9,
            out_specs=pl.BlockSpec(memory_space=pltpu.VMEM),
            out_shape=jax.ShapeDtypeStruct((1, 1, D), BF),
            scratch_shapes=[
                pltpu.VMEM((1, 1, D), BF), pltpu.VMEM((D,), BF),
                pltpu.VMEM((NB, DH, W), BF), pltpu.VMEM((NB, DH, W), BF),
                pltpu.VMEM((D, H * DH), BF), pltpu.VMEM((H * DH, D), BF),
                pltpu.VMEM((D, F), BF), pltpu.VMEM((D, F), BF), pltpu.VMEM((F, D), BF),
                pltpu.VMEM((H, 8, DH), BF), pltpu.VMEM((8, D), F32),
                pltpu.SemaphoreType.DMA((NSEM,)),
            ],
            compiler_params=pltpu.CompilerParams(vmem_limit_bytes=100 * 1024 * 1024,
                                                 disable_semaphore_checks=not semcheck,
                                                 disable_bounds_checks=not bchk),
        )(A_x, gate_w, kT, vT, A_wq, A_wo, B_w1, B_w3, B_w2)
    return f


pallas_gated_mix__sliding_block_cached__glu_gated_swiglu__decode_kernel = make()
```

```python
import jax, jax.numpy as jnp
import jax.experimental.pallas as pl
import jax.experimental.pallas.tpu as pltpu

H, DH, W, D, F = 32, 192, 4096, 640, 1536
BF = jnp.bfloat16
F32 = jnp.float32
NB = 3


def origins(shape, p, r0=0, nr=None, g=1):
    R, C = shape
    nr = R - r0 if nr is None else nr
    assert nr % p[0] == 0 and C % p[1] == 0, (shape, p, nr)
    org = [(r, c) for r in range(r0, r0 + nr, p[0]) for c in range(0, C, p[1])]
    n = len(org)
    assert n % g == 0
    return [org[(i % g) * (n // g) + i // g] for i in range(n)]


def merge(a, b):
    out, n, ia, ib = [], max(len(a), len(b)), 0, 0
    for i in range(n):
        while ia < len(a) and ia * n < (i + 1) * len(a):
            out.append((a[ia], 0)); ia += 1
        while ib < len(b) and ib * n < (i + 1) * len(b):
            out.append((b[ib], 1)); ib += 1
    return out


def make(kv=(192, 128), wq_p=(8, 2048), wo_p=(24, 640), w13_p=(16, 1536), w2_p=(32, 640), tr=(15, 16, 4),
         w2_groups=(512, 512, 384, 128), semcheck=False, bchk=False, frac=0.5, ffn_cuts=(32, 64, 96)):
    assert sum(w2_groups) == F
    w2_offs = [sum(w2_groups[:i]) for i in range(len(w2_groups))]
    NG = len(w2_groups)
    S_K, S_V = 0, NB
    S_X = 2 * NB
    S_GW, S_WQ, S_WO, S_W1, S_W3, S_W2 = S_X + 1, S_X + 2, S_X + 3, S_X + 4, S_X + 5, S_X + 6
    NSEM = S_W2 + NG
    kv_org = [(r, c) for c in range(0, W, kv[1]) for r in range(0, DH, kv[0])]
    cut = int(len(kv_org) * frac)

    def kern(x_hbm, gw_hbm, k_hbm, v_hbm, wq_hbm, wo_hbm, w1_hbm, w3_hbm, w2_hbm, o_ref,
             x_s, gw_s, kbuf, vbuf, wq_s, wo_s, w1_s, w3_s, w2_s, q_s, acc_s, sem):
        SK = k_hbm.shape[3]

        def wpieces(src, dst, p, s, r0=0, nr=None, g=1):
            return [(src, dst, p, s, r, c) for r, c in origins(dst.shape, p, r0, nr, g)]

        def start_w(lst):
            for (src, dst, p, s, r, c), prio in lst:
                pltpu.make_async_copy(src.at[pl.ds(r, p[0]), pl.ds(c, p[1])],
                                      dst.at[pl.ds(r, p[0]), pl.ds(c, p[1])], sem.at[s]).start(priority=prio)

        def wait_all(buf, s):
            pltpu.make_async_copy(buf, buf, sem.at[s]).wait()

        def start_head(h, slot, orgs):
            for r, c in orgs:
                for prio, (src, buf, s) in enumerate(((k_hbm, kbuf, S_K), (v_hbm, vbuf, S_V))):
                    pltpu.make_async_copy(
                        src.at[0, h, pl.ds(r, kv[0]), pl.ds(SK - W + c, kv[1])],
                        buf.at[slot, pl.ds(r, kv[0]), pl.ds(c, kv[1])], sem.at[s + slot]).start(priority=prio)

        ffn = merge(wpieces(w1_hbm, w1_s, w13_p, S_W1, g=tr[2]), wpieces(w3_hbm, w3_s, w13_p, S_W3, g=tr[2]))
        half = F // 2
        for i, (o, n) in enumerate(zip(w2_offs, w2_groups)):
            ps = wpieces(w2_hbm, w2_s, w2_p, S_W2 + i, o, n)
            ffn += merge(ps[:len(ps) // 2], ps[len(ps) // 2:])
        c0, c1, c2 = ffn_cuts

        x_cp = pltpu.make_async_copy(x_hbm, x_s, sem.at[S_X])
        gw_cp = pltpu.make_async_copy(gw_hbm, gw_s, sem.at[S_GW])
        x_cp.start()
        gw_cp.start(priority=1)
        start_w(merge(wpieces(wq_hbm, wq_s, wq_p, S_WQ, g=tr[0]), wpieces(wo_hbm, wo_s, wo_p, S_WO, g=tr[1])))
        start_head(0, 0, kv_org)

        x_cp.wait()
        x = x_s[0]
        x8 = jnp.broadcast_to(x, (8, D))
        wait_all(wq_s, S_WQ)
        for hp in range(H // 2):
            q2 = jnp.dot(x8, wq_s[:, hp * 2 * DH:(hp + 1) * 2 * DH], preferred_element_type=F32)
            q_s[2 * hp] = q2[:, :DH].astype(BF)
            q_s[2 * hp + 1] = q2[:, DH:].astype(BF)
        acc_s[...] = jnp.zeros_like(acc_s)
        wait_all(wo_s, S_WO)
        start_head(1, 1, kv_org[:cut])

        def head(h, carry):
            slot = jax.lax.rem(h, NB)
            wait_all(kbuf.at[slot], S_K + slot)

            @pl.when(h + 1 < H)
            def _():
                start_head(h + 1, jax.lax.rem(h + 1, NB), kv_org[cut:])

            @pl.when(h + 1 == H)
            def _():
                start_w(ffn[c0:c1])

            s = jnp.dot(q_s[h], kbuf[slot], preferred_element_type=F32) * (DH ** -0.5)
            m = jnp.max(s, axis=-1, keepdims=True)
            p = jnp.exp(s - m)
            l = jnp.sum(p, axis=-1, keepdims=True)
            pb = p.astype(BF)
            wait_all(vbuf.at[slot], S_V + slot)

            @pl.when(h + 2 < H)
            def _():
                start_head(h + 2, jax.lax.rem(h + 2, NB), kv_org[:cut])

            @pl.when(h + 2 == H)
            def _():
                start_w(ffn[:c0])

            @pl.when(h + 1 == H)
            def _():
                start_w(ffn[c1:c2])

            o = jax.lax.dot_general(pb, vbuf[slot], (((1,), (1,)), ((), ())), preferred_element_type=F32)
            ob = (o / l).astype(BF)
            row = pl.multiple_of(h * DH, DH)
            acc_s[...] += jnp.dot(ob, wo_s[pl.ds(row, DH), :], preferred_element_type=F32)
            return carry

        jax.lax.fori_loop(0, H, head, 0)
        start_w(ffn[c2:])

        gw_cp.wait()
        gw = gw_s[...].astype(F32).reshape(1, D)
        g = jax.nn.sigmoid(jnp.sum(x.astype(F32) * gw, axis=-1, keepdims=True))
        ga = g * acc_s[...]
        wait_all(w1_s, S_W1)
        gate = jnp.dot(x8, w1_s[...], preferred_element_type=F32)
        sg = gate * jax.nn.sigmoid(gate)
        wait_all(w3_s, S_W3)
        up = jnp.dot(x8, w3_s[...], preferred_element_type=F32)
        hh = (sg * up).astype(BF)
        b = None
        for i, (o, n) in enumerate(zip(w2_offs, w2_groups)):
            wait_all(w2_s.at[pl.ds(o, n)], S_W2 + i)
            part = jnp.dot(hh[:, o:o + n], w2_s[o:o + n, :], preferred_element_type=F32)
            b = part if b is None else b + part
        res = ga + (1 - g) * b
        o_ref[0] = res[0:1].astype(o_ref.dtype)

    @jax.jit
    def f(A_x, A_k_cache, A_v_cache, A_wq, A_wo, B_x, B_w1, B_w3, B_w2, gate_w):
        kT = jnp.swapaxes(A_k_cache, 2, 3)
        vT = jnp.swapaxes(A_v_cache, 2, 3)
        anyspec = pl.BlockSpec(memory_space=pl.ANY)
        return pl.pallas_call(
            kern,
            in_specs=[anyspec] * 9,
            out_specs=pl.BlockSpec(memory_space=pltpu.VMEM),
            out_shape=jax.ShapeDtypeStruct((1, 1, D), BF),
            scratch_shapes=[
                pltpu.VMEM((1, 1, D), BF), pltpu.VMEM((D,), BF),
                pltpu.VMEM((NB, DH, W), BF), pltpu.VMEM((NB, DH, W), BF),
                pltpu.VMEM((D, H * DH), BF), pltpu.VMEM((H * DH, D), BF),
                pltpu.VMEM((D, F), BF), pltpu.VMEM((D, F), BF), pltpu.VMEM((F, D), BF),
                pltpu.VMEM((H, 8, DH), BF), pltpu.VMEM((8, D), F32),
                pltpu.SemaphoreType.DMA((NSEM,)),
            ],
            compiler_params=pltpu.CompilerParams(vmem_limit_bytes=100 * 1024 * 1024,
                                                 disable_semaphore_checks=not semcheck,
                                                 disable_bounds_checks=not bchk),
        )(A_x, gate_w, kT, vT, A_wq, A_wo, B_w1, B_w3, B_w2)
    return f


pallas_gated_mix__sliding_block_cached__glu_gated_swiglu__decode_kernel = make(bchk=True)
```

```python
import jax
import jax.numpy as jnp
import jax.experimental.pallas as pl
import jax.experimental.pallas.tpu as pltpu

BF16 = jnp.bfloat16
F32 = jnp.float32

H, DH, W, D, F = 32, 192, 4096, 640, 1536
NB = 3

KV_P = (64, 256)
WQ_P = (8, 2048)
WO_P = (24, 640)
W13_P = (16, 1536)
W2_P = (32, 640)
W2_SMALL_P = (8, 640)
LAG = 28

W2_MXU = (768, 512)
W2_VPU = (128, 64, 48, 16)
W2_GROUPS = W2_MXU + W2_VPU
W2_OFFS = tuple(sum(W2_GROUPS[:i]) for i in range(len(W2_GROUPS)))
W2_V0 = sum(W2_MXU)
FFN_CUTS = (48, 88, 120)

S_K, S_V = 0, NB
S_X, S_GW, S_WQ, S_WO, S_W1, S_W3, S_W2 = range(2 * NB, 2 * NB + 7)
N_SEM = S_W2 + len(W2_GROUPS)

KV_ORIGINS = [(r, c) for c in range(0, W, KV_P[1]) for r in range(0, DH, KV_P[0])]
KV_HALF = len(KV_ORIGINS) // 2


def _origins(shape, p, r0, nr, streams):
    org = [(r, c) for r in range(r0, r0 + nr, p[0]) for c in range(0, shape[1], p[1])]
    n = len(org)
    assert nr % p[0] == 0 and shape[1] % p[1] == 0 and n % streams == 0
    return [org[(i % streams) * (n // streams) + i // streams] for i in range(n)]


def _merge(a, b):
    out, n, ia, ib = [], max(len(a), len(b)), 0, 0
    for i in range(n):
        while ia < len(a) and ia * n < (i + 1) * len(a):
            out.append((a[ia], 0))
            ia += 1
        while ib < len(b) and ib * n < (i + 1) * len(b):
            out.append((b[ib], 1))
            ib += 1
    return out


def _kernel(x_hbm, gw_hbm, k_hbm, v_hbm, wq_hbm, wo_hbm, w1_hbm, w3_hbm, w2_hbm, o_ref,
            x_s, gw_s, kbuf, vbuf, wq_s, wo_s, w1_s, w3_s, w2_s, q_s, acc_s, sem):
    win0 = k_hbm.shape[3] - W

    def pieces(src, dst, p, s, r0=0, nr=None, streams=1):
        nr = dst.shape[0] if nr is None else nr
        return [(src, dst, p, s, r, c) for r, c in _origins(dst.shape, p, r0, nr, streams)]

    def start(tagged):
        for (src, dst, p, s, r, c), prio in tagged:
            pltpu.make_async_copy(src.at[pl.ds(r, p[0]), pl.ds(c, p[1])],
                                  dst.at[pl.ds(r, p[0]), pl.ds(c, p[1])],
                                  sem.at[s]).start(priority=prio)

    def start_head(h, slot, origins):
        for r, c in origins:
            for prio, (src, buf, s) in enumerate(((k_hbm, kbuf, S_K), (v_hbm, vbuf, S_V))):
                pltpu.make_async_copy(
                    src.at[0, h, pl.ds(r, KV_P[0]), pl.ds(win0 + c, KV_P[1])],
                    buf.at[slot, pl.ds(r, KV_P[0]), pl.ds(c, KV_P[1])],
                    sem.at[s + slot]).start(priority=prio)

    def wait_filled(buf, s):
        pltpu.make_async_copy(buf, buf, sem.at[s]).wait()

    big = (pieces(w1_hbm, w1_s, W13_P, S_W1, streams=4) + pieces(w3_hbm, w3_s, W13_P, S_W3, streams=4))
    small = []
    for i, (o, n) in enumerate(zip(W2_OFFS, W2_GROUPS)):
        if i < len(W2_MXU):
            big += pieces(w2_hbm, w2_s, W2_P, S_W2 + i, o, n, streams=2)
        else:
            small += pieces(w2_hbm, w2_s, W2_SMALL_P, S_W2 + i, o, n)
    ffn = _merge(big[:LAG] + big[LAG::2], big[LAG + 1::2] + small)
    c0, c1, c2 = FFN_CUTS

    x_cp = pltpu.make_async_copy(x_hbm, x_s, sem.at[S_X])
    gw_cp = pltpu.make_async_copy(gw_hbm, gw_s, sem.at[S_GW])
    wq_p = pieces(wq_hbm, wq_s, WQ_P, S_WQ, streams=15)
    wo_p = pieces(wo_hbm, wo_s, WO_P, S_WO, streams=16)
    start([(p, 1) for p in wo_p[:LAG]])
    x_cp.start()
    gw_cp.start()
    start(_merge(wq_p, wo_p[LAG:]))
    start_head(0, 0, KV_ORIGINS)

    x_cp.wait()
    x = x_s[0]
    x8 = jnp.broadcast_to(x, (8, D))
    wait_filled(wq_s, S_WQ)
    for hp in range(H // 2):
        q2 = jnp.dot(x8, wq_s[:, hp * 2 * DH:(hp + 1) * 2 * DH], preferred_element_type=F32)
        q_s[2 * hp] = q2[:, :DH].astype(BF16)
        q_s[2 * hp + 1] = q2[:, DH:].astype(BF16)
    acc_s[...] = jnp.zeros_like(acc_s)
    wait_filled(wo_s, S_WO)
    start_head(1, 1, KV_ORIGINS[:KV_HALF])

    def head(h, carry):
        slot = jax.lax.rem(h, NB)
        wait_filled(kbuf.at[slot], S_K + slot)

        @pl.when(h + 1 < H)
        def _():
            start_head(h + 1, jax.lax.rem(h + 1, NB), KV_ORIGINS[KV_HALF:])

        @pl.when(h + 1 == H)
        def _():
            start(ffn[c0:c1])

        s = jnp.dot(q_s[h], kbuf[slot], preferred_element_type=F32) * (DH ** -0.5)
        m = jnp.max(s, axis=-1, keepdims=True)
        p = jnp.exp(s - m)
        l = jnp.sum(p, axis=-1, keepdims=True)
        pb = p.astype(BF16)
        wait_filled(vbuf.at[slot], S_V + slot)

        @pl.when(h + 2 < H)
        def _():
            start_head(h + 2, jax.lax.rem(h + 2, NB), KV_ORIGINS[:KV_HALF])

        @pl.when(h + 2 == H)
        def _():
            start(ffn[:c0])

        @pl.when(h + 1 == H)
        def _():
            start(ffn[c1:c2])

        o = jax.lax.dot_general(pb, vbuf[slot], (((1,), (1,)), ((), ())),
                                preferred_element_type=F32)
        ob = (o / l).astype(BF16)
        row = pl.multiple_of(h * DH, DH)
        acc_s[...] += jnp.dot(ob, wo_s[pl.ds(row, DH), :], preferred_element_type=F32)
        return carry

    jax.lax.fori_loop(0, H, head, 0)
    start(ffn[c2:])

    gw_cp.wait()
    gw = gw_s[...].astype(F32).reshape(1, D)
    g = jax.nn.sigmoid(jnp.sum(x.astype(F32) * gw, axis=-1, keepdims=True))
    ga = g * acc_s[...]
    wait_filled(w1_s, S_W1)
    gate = jnp.dot(x8, w1_s[...], preferred_element_type=F32)
    act = gate * jax.nn.sigmoid(gate)
    wait_filled(w3_s, S_W3)
    up = jnp.dot(x8, w3_s[...], preferred_element_type=F32)
    hh = (act * up).astype(BF16)
    h_last = hh[0:1, W2_V0:].astype(F32) * (1 - g)
    hcol = jnp.broadcast_to(h_last, (128, F - W2_V0)).T
    b = None
    for i in range(len(W2_MXU)):
        o, n = W2_OFFS[i], W2_GROUPS[i]
        wait_filled(w2_s.at[pl.ds(o, n)], S_W2 + i)
        part = jnp.dot(hh[:, o:o + n], w2_s[o:o + n, :], preferred_element_type=F32)
        b = part if b is None else part + b
    first_row = jax.lax.broadcasted_iota(jnp.int32, (8, D), 0) == 0
    tot = jnp.where(first_row, ga + (1 - g) * b, 0.0)
    for i in range(len(W2_MXU), len(W2_GROUPS)):
        o, n = W2_OFFS[i], W2_GROUPS[i]
        wait_filled(w2_s.at[pl.ds(o, n)], S_W2 + i)
        hc = hcol[o - W2_V0:o - W2_V0 + n, :]
        prod = w2_s[o:o + n, :].astype(F32) * jnp.concatenate([hc] * (D // 128), axis=1)
        tot = tot + jnp.sum(prod.reshape(n // 8, 8, D), axis=0)
    o_ref[0] = jnp.sum(tot, axis=0, keepdims=True).astype(o_ref.dtype)


@jax.jit
def pallas_gated_mix__sliding_block_cached__glu_gated_swiglu__decode_kernel(
    A_x: jax.Array,
    A_k_cache: jax.Array,
    A_v_cache: jax.Array,
    A_wq: jax.Array,
    A_wo: jax.Array,
    B_x: jax.Array,
    B_w1: jax.Array,
    B_w3: jax.Array,
    B_w2: jax.Array,
    gate_w: jax.Array,
):
    del B_x
    assert A_x.shape == (1, 1, D) and A_k_cache.shape[:2] == (1, H) and A_k_cache.shape[3] == DH
    assert min(4096, max(256, A_k_cache.shape[2] // 4)) == W
    k_t = jnp.swapaxes(A_k_cache, 2, 3)
    v_t = jnp.swapaxes(A_v_cache, 2, 3)
    params = dict(vmem_limit_bytes=64 * 1024 * 1024)
    if hasattr(pltpu.CompilerParams, "disable_semaphore_checks"):
        params["disable_semaphore_checks"] = True
    return pl.pallas_call(
        _kernel,
        in_specs=[pl.BlockSpec(memory_space=pl.ANY)] * 9,
        out_specs=pl.BlockSpec(memory_space=pltpu.VMEM),
        out_shape=jax.ShapeDtypeStruct((1, 1, D), A_x.dtype),
        scratch_shapes=[
            pltpu.VMEM((1, 1, D), BF16), pltpu.VMEM((D,), BF16),
            pltpu.VMEM((NB, DH, W), BF16), pltpu.VMEM((NB, DH, W), BF16),
            pltpu.VMEM((D, H * DH), BF16), pltpu.VMEM((H * DH, D), BF16),
            pltpu.VMEM((D, F), BF16), pltpu.VMEM((D, F), BF16), pltpu.VMEM((F, D), BF16),
            pltpu.VMEM((H, 8, DH), BF16), pltpu.VMEM((8, D), F32),
            pltpu.SemaphoreType.DMA((N_SEM,)),
        ],
        compiler_params=pltpu.CompilerParams(**params),
    )(A_x, gate_w, k_t, v_t, A_wq, A_wo, B_w1, B_w3, B_w2)
```

```python
import jax
import jax.numpy as jnp
import jax.experimental.pallas as pl
import jax.experimental.pallas.tpu as pltpu

BF16 = jnp.bfloat16
F32 = jnp.float32

H, DH, W, D, F = 32, 192, 4096, 640, 1536
NB = 3

WQ_SHAPE = (5, D // 5, H * DH)
WO_SHAPE = (1, H * DH, D)
W13_SHAPE = (4, D // 4, F)
W2_SHAPE = (1, F, D)

KV_P = (64, 256)
WQ_P = (5, 8, 384)
WO_P = (1, 24, 640)
W13_P = (4, 8, 512)
W2_P = (1, 32, 640)
W2_SMALL_P = (1, 8, 640)
LAG = 28

W2_MXU = (768, 512)
W2_VPU = (128, 64, 48, 16)
W2_GROUPS = W2_MXU + W2_VPU
W2_OFFS = tuple(sum(W2_GROUPS[:i]) for i in range(len(W2_GROUPS)))
W2_V0 = sum(W2_MXU)
FFN_CUTS = (48, 96, 144)

S_K, S_V = 0, NB
S_X, S_GW, S_WQ, S_WO, S_W1, S_W3, S_W2 = range(2 * NB, 2 * NB + 7)
N_SEM = S_W2 + len(W2_GROUPS)

KV_ORIGINS = [(r, c) for c in range(0, W, KV_P[1]) for r in range(0, DH, KV_P[0])]
KV_HALF = len(KV_ORIGINS) // 2


def _origins(shape, p, r0, nr, streams):
    groups, _, cols = shape
    org = [(g, r, c) for r in range(r0, r0 + nr, p[1]) for c in range(0, cols, p[2])
           for g in range(0, groups, p[0])]
    n = len(org)
    assert groups % p[0] == 0 and nr % p[1] == 0 and cols % p[2] == 0 and n % streams == 0
    return [org[(i % streams) * (n // streams) + i // streams] for i in range(n)]


def _merge(a, b):
    out, n, ia, ib = [], max(len(a), len(b)), 0, 0
    for i in range(n):
        while ia < len(a) and ia * n < (i + 1) * len(a):
            out.append((a[ia], 0))
            ia += 1
        while ib < len(b) and ib * n < (i + 1) * len(b):
            out.append((b[ib], 1))
            ib += 1
    return out


def _kernel(x_hbm, gw_hbm, k_hbm, v_hbm, wq_hbm, wo_hbm, w1_hbm, w3_hbm, w2_hbm, o_ref,
            x_s, gw_s, kbuf, vbuf, wq_s, wo_s, w1_s, w3_s, w2_s, q_s, acc_s, sem):
    win0 = k_hbm.shape[3] - W

    def pieces(src, dst, p, s, r0=0, nr=None, streams=1):
        nr = dst.shape[1] if nr is None else nr
        return [(src, dst, p, s, o) for o in _origins(dst.shape, p, r0, nr, streams)]

    def start(tagged):
        for (src, dst, p, s, origin), prio in tagged:
            idx = tuple(pl.ds(a, n) for a, n in zip(origin, p))
            pltpu.make_async_copy(src.at[idx], dst.at[idx], sem.at[s]).start(priority=prio)

    def start_head(h, slot, origins):
        for r, c in origins:
            for prio, (src, buf, s) in enumerate(((k_hbm, kbuf, S_K), (v_hbm, vbuf, S_V))):
                pltpu.make_async_copy(
                    src.at[0, h, pl.ds(r, KV_P[0]), pl.ds(win0 + c, KV_P[1])],
                    buf.at[slot, pl.ds(r, KV_P[0]), pl.ds(c, KV_P[1])],
                    sem.at[s + slot]).start(priority=prio)

    def wait_filled(buf, s):
        pltpu.make_async_copy(buf, buf, sem.at[s]).wait()

    big = pieces(w1_hbm, w1_s, W13_P, S_W1) + pieces(w3_hbm, w3_s, W13_P, S_W3)
    small = []
    for i, (o, n) in enumerate(zip(W2_OFFS, W2_GROUPS)):
        if i < len(W2_MXU):
            big += pieces(w2_hbm, w2_s, W2_P, S_W2 + i, o, n, streams=2)
        else:
            small += pieces(w2_hbm, w2_s, W2_SMALL_P, S_W2 + i, o, n)
    ffn = _merge(big[:LAG] + big[LAG::2], big[LAG + 1::2] + small)
    c0, c1, c2 = FFN_CUTS

    x_cp = pltpu.make_async_copy(x_hbm, x_s, sem.at[S_X])
    gw_cp = pltpu.make_async_copy(gw_hbm, gw_s, sem.at[S_GW])
    wq_p = pieces(wq_hbm, wq_s, WQ_P, S_WQ)
    wo_p = pieces(wo_hbm, wo_s, WO_P, S_WO, streams=8)
    start([(p, 1) for p in wo_p[:LAG]])
    x_cp.start()
    gw_cp.start()
    start(_merge(wq_p, wo_p[LAG:]))
    start_head(0, 0, KV_ORIGINS)

    x_cp.wait()
    x = x_s[0]
    x8 = jnp.broadcast_to(x, (8, D))
    wait_filled(wq_s, S_WQ)
    for hp in range(H // 2):
        wq2 = wq_s[:, :, hp * 2 * DH:(hp + 1) * 2 * DH].reshape(D, 2 * DH)
        q2 = jnp.dot(x8, wq2, preferred_element_type=F32)
        q_s[2 * hp] = q2[:, :DH].astype(BF16)
        q_s[2 * hp + 1] = q2[:, DH:].astype(BF16)
    acc_s[...] = jnp.zeros_like(acc_s)
    wait_filled(wo_s, S_WO)
    start_head(1, 1, KV_ORIGINS[:KV_HALF])

    def head(h, carry):
        slot = jax.lax.rem(h, NB)
        wait_filled(kbuf.at[slot], S_K + slot)

        @pl.when(h + 1 < H)
        def _():
            start_head(h + 1, jax.lax.rem(h + 1, NB), KV_ORIGINS[KV_HALF:])

        @pl.when(h + 1 == H)
        def _():
            start(ffn[c0:c1])

        s = jnp.dot(q_s[h], kbuf[slot], preferred_element_type=F32) * (DH ** -0.5)
        m = jnp.max(s, axis=-1, keepdims=True)
        p = jnp.exp(s - m)
        l = jnp.sum(p, axis=-1, keepdims=True)
        pb = p.astype(BF16)
        wait_filled(vbuf.at[slot], S_V + slot)

        @pl.when(h + 2 < H)
        def _():
            start_head(h + 2, jax.lax.rem(h + 2, NB), KV_ORIGINS[:KV_HALF])

        @pl.when(h + 2 == H)
        def _():
            start(ffn[:c0])

        @pl.when(h + 1 == H)
        def _():
            start(ffn[c1:c2])

        o = jax.lax.dot_general(pb, vbuf[slot], (((1,), (1,)), ((), ())),
                                preferred_element_type=F32)
        ob = (o / l).astype(BF16)
        row = pl.multiple_of(h * DH, DH)
        acc_s[...] += jnp.dot(ob, wo_s[0, pl.ds(row, DH), :], preferred_element_type=F32)
        return carry

    jax.lax.fori_loop(0, H, head, 0)
    start(ffn[c2:])

    gw_cp.wait()
    gw = gw_s[...].astype(F32).reshape(1, D)
    g = jax.nn.sigmoid(jnp.sum(x.astype(F32) * gw, axis=-1, keepdims=True))
    ga = g * acc_s[...]
    wait_filled(w1_s, S_W1)
    gate = jnp.dot(x8, w1_s[...].reshape(D, F), preferred_element_type=F32)
    act = gate * jax.nn.sigmoid(gate)
    wait_filled(w3_s, S_W3)
    up = jnp.dot(x8, w3_s[...].reshape(D, F), preferred_element_type=F32)
    hh = (act * up).astype(BF16)
    h_last = hh[0:1, W2_V0:].astype(F32) * (1 - g)
    hcol = jnp.broadcast_to(h_last, (128, F - W2_V0)).T
    b = None
    for i in range(len(W2_MXU)):
        o, n = W2_OFFS[i], W2_GROUPS[i]
        wait_filled(w2_s.at[:, pl.ds(o, n)], S_W2 + i)
        part = jnp.dot(hh[:, o:o + n], w2_s[0, o:o + n, :], preferred_element_type=F32)
        b = part if b is None else part + b
    first_row = jax.lax.broadcasted_iota(jnp.int32, (8, D), 0) == 0
    tot = jnp.where(first_row, ga + (1 - g) * b, 0.0)
    for i in range(len(W2_MXU), len(W2_GROUPS)):
        o, n = W2_OFFS[i], W2_GROUPS[i]
        wait_filled(w2_s.at[:, pl.ds(o, n)], S_W2 + i)
        hc = hcol[o - W2_V0:o - W2_V0 + n, :]
        prod = w2_s[0, o:o + n, :].astype(F32) * jnp.concatenate([hc] * (D // 128), axis=1)
        tot = tot + jnp.sum(prod.reshape(n // 8, 8, D), axis=0)
    o_ref[0] = jnp.sum(tot, axis=0, keepdims=True).astype(o_ref.dtype)


@jax.jit
def pallas_gated_mix__sliding_block_cached__glu_gated_swiglu__decode_kernel(
    A_x: jax.Array,
    A_k_cache: jax.Array,
    A_v_cache: jax.Array,
    A_wq: jax.Array,
    A_wo: jax.Array,
    B_x: jax.Array,
    B_w1: jax.Array,
    B_w3: jax.Array,
    B_w2: jax.Array,
    gate_w: jax.Array,
):
    del B_x
    assert A_x.shape == (1, 1, D) and A_k_cache.shape[:2] == (1, H) and A_k_cache.shape[3] == DH
    assert min(4096, max(256, A_k_cache.shape[2] // 4)) == W
    k_t = jnp.swapaxes(A_k_cache, 2, 3)
    v_t = jnp.swapaxes(A_v_cache, 2, 3)
    params = dict(vmem_limit_bytes=64 * 1024 * 1024)
    if hasattr(pltpu.CompilerParams, "disable_semaphore_checks"):
        params["disable_semaphore_checks"] = True
    return pl.pallas_call(
        _kernel,
        in_specs=[pl.BlockSpec(memory_space=pl.ANY)] * 9,
        out_specs=pl.BlockSpec(memory_space=pltpu.VMEM),
        out_shape=jax.ShapeDtypeStruct((1, 1, D), A_x.dtype),
        scratch_shapes=[
            pltpu.VMEM((1, 1, D), BF16), pltpu.VMEM((D,), BF16),
            pltpu.VMEM((NB, DH, W), BF16), pltpu.VMEM((NB, DH, W), BF16),
            pltpu.VMEM(WQ_SHAPE, BF16), pltpu.VMEM(WO_SHAPE, BF16),
            pltpu.VMEM(W13_SHAPE, BF16), pltpu.VMEM(W13_SHAPE, BF16), pltpu.VMEM(W2_SHAPE, BF16),
            pltpu.VMEM((H, 8, DH), BF16), pltpu.VMEM((8, D), F32),
            pltpu.SemaphoreType.DMA((N_SEM,)),
        ],
        compiler_params=pltpu.CompilerParams(**params),
    )(A_x, gate_w, k_t, v_t, A_wq.reshape(WQ_SHAPE), A_wo.reshape(WO_SHAPE),
      B_w1.reshape(W13_SHAPE), B_w3.reshape(W13_SHAPE), B_w2.reshape(W2_SHAPE))
```
